```python
import os as _os
_os.environ.setdefault("JAX_PLATFORMS", "cpu")
import jax
import jax.numpy as jnp

def _softmax(x, axis=-1):
    return jax.nn.softmax(x, axis=axis)
def _gelu(x):
    return jax.nn.gelu(x, approximate=True)
def _silu(x):
    return jax.nn.silu(x)
def _sigmoid(x):
    return jax.nn.sigmoid(x)
def _layernorm(x, axis=-1, eps=1e-5):
    m = jnp.mean(x, axis=axis, keepdims=True)
    v = jnp.var(x, axis=axis, keepdims=True)
    return (x - m) / jnp.sqrt(v + eps)
def _scatter_add(tgt, idx, src, axis=0):
    return tgt.at[idx].add(src)
def _segment_sum(src, seg, n):
    return jax.ops.segment_sum(src, seg, n)
class _Rng:
    def __init__(self, key):
        self._k = key
    def _next(self):
        self._k, sub = jax.random.split(self._k)
        return sub
    def normal(self, shape):
        return jax.random.normal(self._next(), shape, dtype=jnp.bfloat16)
    def randint(self, lo, hi, shape):
        return jax.random.randint(self._next(), shape, lo, hi, dtype=jnp.int32)
    def uniform(self, shape, lo=0.0, hi=1.0):
        return jax.random.uniform(self._next(), shape, jnp.bfloat16, lo, hi)
    def permutation(self, n):
        return jax.random.permutation(self._next(), n)


kernel_name = 'standalone__geglu_ffn__prompt'

def setup_inputs():
    _rng = _Rng(jax.random.key(int.from_bytes(__import__("os").urandom(4), "little")))
    _w = (lambda a: (lambda t: t.astype(jnp.bfloat16) if jnp.issubdtype(t.dtype, jnp.floating) else t)(jnp.asarray(a)))
    B, S, D, F = 1, 2048, 576, 4608
    return {
        "x": _w((lambda *s: _rng.normal(s) * 0.05)(B, S, D)),
        "w_gate": _w((lambda *s: _rng.normal(s) * 0.05)(D, F)),
        "w_up": _w((lambda *s: _rng.normal(s) * 0.05)(D, F)),
        "w_down": _w((lambda *s: _rng.normal(s) * 0.05)(F, D)),
    }

def reference(x, w_gate, w_up, w_down):
    return (_gelu(x @ w_gate) * (x @ w_up)) @ w_down
```

```python
import contextlib
import jax, jax.numpy as jnp, numpy as np
from jax import lax
from jax.experimental import pallas as pl
from jax.experimental.pallas import tpu as pltpu

C0 = float(np.sqrt(2/np.pi)); C1 = float(np.sqrt(2/np.pi)*0.044715)
def geglu(g, u):
    t = jnp.tanh(g*(C0 + C1*(g*g)))
    return (0.5*g)*(1.0+t)*u

def cum(sizes, o=0):
    r = []
    for s in sizes:
        r.append((o, s)); o += s
    return r

NT = (((1,), (1,)), ((), ()))
f32 = jnp.float32

def make(FA=128, FB=256, NH=2, FU=(512, 512, 384), OUT=(256, 256), XP=2, scopes=False, vmem=100, flags=None, nochk=True, SB=512, order="sf"):
    F0 = FA + FB; FM = sum(FU)
    def kernel(xT_hbm, wg_hbm, wu_hbm, wdT_hbm, oT_hbm, xT_v, x_v, wg0, wu0, wd0, wg, wu, wd, acc, o_v, xsem, w0sem, wsem, osem):
        ns = (lambda n: jax.named_scope(n)) if scopes else (lambda n: contextlib.nullcontext())
        D, S = xT_hbm.shape; F = wg_hbm.shape[1]
        NC = S // SB; H = SB // XP; NB = (F - F0) // FM; CPH = NC // NH
        cp = pltpu.make_async_copy
        x0 = [cp(xT_hbm.at[:, pl.ds(c*H, H)], xT_v.at[0, :, pl.ds(c*H, H)], xsem.at[c]) for c in range(XP)]
        xr = [None] + [cp(xT_hbm.at[:, pl.ds(c*SB, SB)], xT_v.at[c], xsem.at[XP-1+c]) for c in range(1, NC)]
        wa = [cp(s.at[:, pl.ds(0, FA)], d.at[:, pl.ds(0, FA)], w0sem.at[k]) for k, (s, d) in enumerate(((wg_hbm, wg0), (wu_hbm, wu0)))]
        wb = [cp(s.at[:, pl.ds(FA, FB)], d.at[:, pl.ds(FA, FB)], w0sem.at[2+k]) for k, (s, d) in enumerate(((wg_hbm, wg0), (wu_hbm, wu0)))]
        wc = cp(wdT_hbm.at[:, pl.ds(0, F0)], wd0, w0sem.at[4])
        def wm(j):
            return [cp(s.at[:, pl.ds(F0 + j*FM, FM)], d.at[j], wsem.at[j])
                    for s, d in ((wg_hbm, wg), (wu_hbm, wu), (wdT_hbm, wd))]
        def gate_up(xs, wg_, wu_):
            g = jnp.dot(xs, wg_, preferred_element_type=f32)
            u = jnp.dot(xs, wu_, preferred_element_type=f32)
            return geglu(g, u).astype(jnp.bfloat16)
        def down(h, wd_):
            return lax.dot_general(wd_, h, NT, preferred_element_type=f32)
        def ocp(c, o, n):
            off = c*SB + o
            if not isinstance(c, int): off = pl.multiple_of(off, 128)
            return cp(o_v.at[c, :, pl.ds(o, n)], oT_hbm.at[:, pl.ds(off, n)], osem)
        for c in x0: c.start()
        for c in wa: c.start()
        for c in range(XP):
            with ns("xwait"):
                x0[c].wait()
            if c == XP-1:
                for d in wb: d.start()
            with ns("xT"):
                x_v[0, c*H:(c+1)*H, :] = xT_v[0, :, c*H:(c+1)*H].T
        with ns("wa"):
            for c in wa: c.wait()
        wc.start(); xr[1].start()
        with ns("gu_a"):
            ha = jnp.concatenate([gate_up(x_v[0, q*256:(q+1)*256, :], wg0[:, :FA], wu0[:, :FA]) for q in range(2)], axis=0)
        with ns("wb"):
            for c in wb: c.wait()
        for c in xr[2:]: c.start()
        with ns("gu_b"):
            hb = gate_up(x_v[0], wg0[:, FA:], wu0[:, FA:])
        with ns("wc"):
            wc.wait(); xr[1].wait()
        for c in wm(0): c.start()
        with ns("p0_1"):
            x_v[1] = xT_v[1].T
            acc[0] = down(jnp.concatenate([ha, hb], axis=1), wd0[...])
            hb = gate_up(x_v[1], wg0[:, FA:], wu0[:, FA:])
        with ns("xr"):
            for c in xr[2:]: c.wait()
        with ns("p0_2"):
            ha = jnp.concatenate([gate_up(x_v[1, q*256:(q+1)*256, :], wg0[:, :FA], wu0[:, :FA]) for q in range(2)], axis=0)
            h = jnp.concatenate([ha, hb], axis=1)
            for c in range(2, NC):
                x_v[c] = xT_v[c].T
                acc[c-1] = down(h, wd0[...])
                h = gate_up(x_v[c], wg0[...], wu0[...])
            acc[NC-1] = down(h, wd0[...])
        def body(it, carry):
            j = it // NH; hf = it % NH
            @pl.when(hf == 0)
            def _():
                for c in wm_dyn(j): c.wait()
                @pl.when(j + 1 < NB)
                def _():
                    for c in wm_dyn(j+1): c.start()
            steps = [(c, k) for c in range(CPH) for k in range(len(FU))]
            with ns("body"):
              for (c, k) in steps:
                o, n = cum(FU)[k]
                ci = hf*CPH + c
                h = gate_up(x_v[ci], wg[j, :, o:o+n], wu[j, :, o:o+n])
                if k < len(FU)-1:
                    acc[ci] += down(h, wd[j, :, o:o+n])
                else:
                    for (so, sn) in (cum(OUT) if c == CPH-1 else [(0, SB)]):
                        val = acc[ci, :, so:so+sn] + down(h[so:so+sn], wd[j, :, o:o+n])
                        acc[ci, :, so:so+sn] = val
                        o_v[ci, :, so:so+sn] = val.astype(o_v.dtype)
                        @pl.when(j == NB-1)
                        def _():
                            ocp(ci, so, sn).start()
            return carry
        def wm_dyn(j):
            off = pl.multiple_of(F0 + j*FM, 128)
            return [cp(s.at[:, pl.ds(off, FM)], d.at[j], wsem.at[j])
                    for s, d in ((wg_hbm, wg), (wu_hbm, wu), (wdT_hbm, wd))]
        lax.fori_loop(0, NB*NH, body, 0)
        with ns("owait"):
            for ci in range(NC):
                for (so, sn) in (cum(OUT) if ci % CPH == CPH-1 else [(0, SB)]):
                    ocp(ci, so, sn).wait()

    def fn(x, wg, wu, wd):
        B, S, D = x.shape; F = wg.shape[1]
        NB = (F - F0)//FM
        assert F0 + NB*FM == F
        xT = x.reshape(S, D).T
        wdT = wd.T
        bf = jnp.bfloat16
        NC = S // SB
        scr = [pltpu.VMEM((NC, D, SB), bf), pltpu.VMEM((NC, SB, D), bf)] + [pltpu.VMEM((D, F0), bf)]*3 + [pltpu.VMEM((NB, D, FM), bf)]*3 \
            + [pltpu.VMEM((NC, D, SB), f32), pltpu.VMEM((NC, D, SB), bf),
               pltpu.SemaphoreType.DMA((XP+NC-1,)), pltpu.SemaphoreType.DMA((5,)), pltpu.SemaphoreType.DMA((NB,)), pltpu.SemaphoreType.DMA(())]
        oT = pl.pallas_call(
            kernel,
            in_specs=[pl.BlockSpec(memory_space=pl.ANY)]*4,
            out_specs=pl.BlockSpec(memory_space=pl.ANY),
            out_shape=jax.ShapeDtypeStruct((D, S), x.dtype),
            scratch_shapes=scr,
            compiler_params=pltpu.CompilerParams(vmem_limit_bytes=vmem*1024*1024, disable_bounds_checks=nochk, **({"flags": flags} if flags else {})),
        )(xT, wg, wu, wdT)
        return oT.T.reshape(B, S, D)
    return fn


@jax.jit
def pallas_standalone__geglu_ffn__prompt_kernel(x, w_gate, w_up, w_down):
    return make()(x, w_gate, w_up, w_down)
```

```python
import jax
import jax.numpy as jnp
import numpy as np
from jax import lax
from jax.experimental import pallas as pl
from jax.experimental.pallas import tpu as pltpu

_C0 = float(np.sqrt(2.0 / np.pi))
_C1 = float(np.sqrt(2.0 / np.pi) * 0.044715)
_F32 = jnp.float32
_BF16 = jnp.bfloat16


def _spans(sizes):
    out, off = [], 0
    for n in sizes:
        out.append((off, n))
        off += n
    return out


def _mm(a, b):
    return jnp.dot(a, b, preferred_element_type=_F32)


def _mm_nt(a, b):
    return lax.dot_general(a, b, (((1,), (1,)), ((), ())), preferred_element_type=_F32)


def _act2(g, u):
    t = jnp.tanh(g * (_C0 + _C1 * (g * g)))
    return ((g * (1.0 + t)) * u).astype(_BF16)


def make(FU=(128, 256, 256, 256, 512), OUT=(256, 128, 128), VR=80, M=(0,), red=True, P0V=(), nosem=False):
    SB = 512
    H = 256
    FA, FB = 256, 128
    NH = 2
    KM = 512
    F0, FM = FA + FB, sum(FU)

    def kernel(xT_hbm, wg_hbm, wu_hbm, wdT_hbm, oT_hbm,
               xT_v, x_v, wg0, wu0, wd0, wg, wu, wd, acc, o_v, xs, zs, zv, psem, wsem, osem):
        D, S = xT_hbm.shape
        F = wg_hbm.shape[1]
        NC, NB, KR = S // SB, (F - F0) // FM, D - KM
        CPH = NC // NH

        def cols(src, dst, off, n, sem):
            return pltpu.make_async_copy(src.at[:, pl.ds(off, n)], dst.at[:, pl.ds(off, n)], psem.at[sem])

        def x_chunk(c, sem):
            return pltpu.make_async_copy(xT_hbm.at[:, pl.ds(c * SB, SB)], xT_v.at[c], psem.at[sem])

        def w_block(j):
            off = F0 + j * FM
            if not isinstance(j, int):
                off = pl.multiple_of(off, 128)
            return [pltpu.make_async_copy(s.at[:, pl.ds(off, FM)], d.at[j], wsem.at[j])
                    for s, d in ((wg_hbm, wg), (wu_hbm, wu), (wdT_hbm, wd))]

        def out_piece(c, off, n):
            dst = c * SB + off
            if not isinstance(c, int):
                dst = pl.multiple_of(dst, 128)
            return pltpu.make_async_copy(o_v.at[c, :, pl.ds(off, n)], oT_hbm.at[:, pl.ds(dst, n)], osem)

        def start(copies):
            for c in copies:
                c.start()

        def wait(copies):
            for c in copies:
                c.wait()

        def transpose_x(c, off, n):
            x_v[c, off:off + n, :] = xT_v[c, :, off:off + n].T

        def gate_up(x, w_g, w_u):
            return _act2(_mm(x, w_g), _mm(x, w_u))

        def skew_x(c):
            xt = xT_v[c, KM:, 0:128].astype(_F32)
            k = lax.broadcasted_iota(jnp.int32, (KR, 128), 0)
            lane = lax.broadcasted_iota(jnp.int32, (KR, 128), 1)
            for i in range(8):
                rel = lane - ((k - i) & 7)
                for r in range(VR // 8):
                    if red:
                        picked = jnp.sum(jnp.where(rel == 8 * r, xt, 0.0), axis=1, keepdims=True)
                        xs[c, r, i] = jnp.broadcast_to(picked, (KR, 128))
                    else:
                        xs[c, r, i] = jnp.take_along_axis(xt, 8 * r + ((k - i) & 7), axis=1)

        def vpu_tail(c, w, prev):
            never = zv[...] != 0
            rows = []
            for r in range(0, VR // 8, 2):
                a = [None, None]
                for i in range(7, -1, -1):
                    m, kb, groups = M[i % len(M)], 0, []
                    for t in range(8 - m):
                        n = 2 if (t * m) % (8 - m) < m else 1
                        groups.append(range(kb, kb + n))
                        kb += n
                    for kbs in groups:
                        for q in range(2):
                            p = [xs[c, r + q, i, 8 * b:8 * b + 8, :] * w[8 * b:8 * b + 8] for b in kbs]
                            p = p[0] if len(p) == 1 else p[0] + p[1]
                            if a[q] is not None:
                                a[q] = a[q] + p
                            elif prev[0] is None:
                                a[q] = p
                            else:
                                a[q] = jnp.where(never, prev[0][q], p)
                    if i:
                        a = [pltpu.roll(v, 7, 0) for v in a]
                prev[0] = a
                rows += a
            return jnp.concatenate(rows, axis=0)

        def project(c, w_at, off, n, prev):
            main = _mm(x_v[c, :, :KM], w_at(False)[:KM, off:off + n])
            tail = _mm(x_v[c, VR:, KM:], w_at(False)[KM:, off:off + n])
            tiles = [(t, w_at(True)[KM:, t:t + 128].astype(_F32)) for t in range(off, off + n, 128)]
            return main, tail, tiles

        def gate_up_split(c, g_at, u_at, off, n, prev):
            gm, gt, gw = project(c, g_at, off, n, prev)
            um, ut, uw = project(c, u_at, off, n, prev)
            gv, uv = [], []
            for (_, a), (_, b) in zip(gw, uw):
                gv.append(vpu_tail(c, a, prev))
                uv.append(vpu_tail(c, b, prev))
            g = gm + jnp.concatenate([jnp.concatenate(gv, axis=1), gt], axis=0)
            u = um + jnp.concatenate([jnp.concatenate(uv, axis=1), ut], axis=0)
            return _act2(g, u)

        xa = cols(xT_hbm, xT_v.at[0], 0, H, 0)
        ga = cols(wg_hbm, wg0, 0, FA, 1)
        ua = cols(wu_hbm, wu0, 0, FA, 2)
        g2 = [cols(xT_hbm, xT_v.at[0], H, H, 3), cols(wg_hbm, wg0, FA, FB, 3), cols(wu_hbm, wu0, FA, FB, 3)]
        g3 = [cols(wdT_hbm, wd0, 0, F0, 4), x_chunk(1, 4)]
        g4 = [x_chunk(c, 5) for c in range(2, NC)]

        start([xa, ga, ua])
        zv[...] = jnp.zeros_like(zv)
        for i in range(zs.shape[0]):
            zs[i] = 0
        xa.wait()
        start(g2)
        transpose_x(0, 0, H)
        ga.wait()
        start(g3)
        g = jnp.concatenate([_mm(x_v[0, o:o + 128], wg0[:, :FA]) for o in range(0, H, 128)], axis=0)
        ua.wait()
        u = jnp.concatenate([_mm(x_v[0, o:o + 128], wu0[:, :FA]) for o in range(0, H, 128)], axis=0)
        h00 = _act2(g, u)
        wait(g2)
        start(g4)
        transpose_x(0, H, H)
        h01 = gate_up(x_v[0, :H], wg0[:, FA:], wu0[:, FA:])
        h1 = gate_up(x_v[0, H:], wg0[...], wu0[...])
        h = jnp.concatenate([jnp.concatenate([h00, h01], axis=1), h1], axis=0)
        wait(g3)
        start(w_block(0))
        transpose_x(1, 0, SB)
        acc[0] = _mm_nt(wd0[...], h)
        ha = gate_up(x_v[1], wg0[:, :FA], wu0[:, :FA])
        wait(g4)
        for c in list(P0V) + [c for c in range(NC) if c not in P0V]:
            skew_x(c)
        prev = [None]
        for c in range(1, NC):
            if c == 1:
                hb = [gate_up(x_v[c, o:o + H], wg0[:, FA:], wu0[:, FA:]) for o in range(0, SB, H)]
                h = jnp.concatenate([ha, jnp.concatenate(hb, axis=0)], axis=1)
            elif c in P0V:
                h = gate_up_split(c, lambda fresh: wg0, lambda fresh: wu0, 0, F0, prev)
            else:
                h = gate_up(x_v[c], wg0[...], wu0[...])
            if c + 1 < NC:
                transpose_x(c + 1, 0, SB)
            acc[c] = _mm_nt(wd0[...], h)

        def body(it, carry):
            j, half = it // NH, it % NH

            @pl.when(half == 0)
            def _():
                wait(w_block(j))

                @pl.when(j + 1 < NB)
                def _():
                    start(w_block(j + 1))

            count = [0]

            def view(ref):
                def at(fresh):
                    if not fresh:
                        return ref.at[j]
                    count[0] += 1
                    return ref.at[j + zs[count[0] % zs.shape[0]]]
                return at

            def down(c, k, h):
                off, n = _spans(FU)[k]
                ci = half * CPH + c
                if k < len(FU) - 1:
                    acc[ci] += _mm_nt(wd[j, :, off:off + n], h)
                    return
                for so, sn in _spans(OUT if c == CPH - 1 else (SB,)):
                    val = acc[ci, :, so:so + sn] + _mm_nt(wd[j, :, off:off + n], h[so:so + sn])
                    acc[ci, :, so:so + sn] = val
                    o_v[ci, :, so:so + sn] = (0.5 * val).astype(o_v.dtype)

                    @pl.when(j == NB - 1)
                    def _():
                        out_piece(ci, so, sn).start()

            prev, pending = [None], None
            for c in range(CPH):
                for k, (off, n) in enumerate(_spans(FU)):
                    h = gate_up_split(half * CPH + c, view(wg), view(wu), off, n, prev)
                    if pending is not None:
                        down(*pending)
                    pending = (c, k, h)
            down(*pending)
            return carry

        lax.fori_loop(0, NB * NH, body, 0)
        for c in range(NC):
            wait([out_piece(c, so, sn) for so, sn in _spans(OUT if c % CPH == CPH - 1 else (SB,))])

    def fn(x, w_gate, w_up, w_down):
        B, S, D = x.shape
        F = w_gate.shape[1]
        T = B * S
        NB, NC = (F - F0) // FM, T // SB
        assert F0 + NB * FM == F and NC * SB == T and NC % NH == 0 and D - KM == 64
        scratch = (
            [pltpu.VMEM((NC, D, SB), _BF16), pltpu.VMEM((NC, SB, D), _BF16)]
            + [pltpu.VMEM((D, F0), _BF16)] * 3
            + [pltpu.VMEM((NB, D, FM), _BF16)] * 3
            + [pltpu.VMEM((NC, D, SB), _F32), pltpu.VMEM((NC, D, SB), x.dtype),
               pltpu.VMEM((NC, VR // 8, 8, D - KM, 128), _F32),
               pltpu.SMEM((16,), jnp.int32), pltpu.VMEM((8, 128), jnp.int32),
               pltpu.SemaphoreType.DMA((6,)), pltpu.SemaphoreType.DMA((NB,)), pltpu.SemaphoreType.DMA(())]
        )
        out_t = pl.pallas_call(
            kernel,
            in_specs=[pl.BlockSpec(memory_space=pl.ANY)] * 4,
            out_specs=pl.BlockSpec(memory_space=pl.ANY),
            out_shape=jax.ShapeDtypeStruct((D, T), x.dtype),
            scratch_shapes=scratch,
            compiler_params=pltpu.CompilerParams(
                vmem_limit_bytes=100 * 1024 * 1024, disable_bounds_checks=True,
                disable_semaphore_checks=nosem),
        )(x.reshape(T, D).T, w_gate, w_up, w_down.T)
        return out_t.T.reshape(B, S, D)

    return fn


@jax.jit
def pallas_standalone__geglu_ffn__prompt_kernel(x, w_gate, w_up, w_down):
    return make()(x, w_gate, w_up, w_down)
```

```python
import jax
import jax.numpy as jnp
import numpy as np
from jax import lax
from jax.experimental import pallas as pl
from jax.experimental.pallas import tpu as pltpu

_C0 = float(np.sqrt(2.0 / np.pi))
_C1 = float(np.sqrt(2.0 / np.pi) * 0.044715)
_F32 = jnp.float32
_BF16 = jnp.bfloat16

_SB = 512
_HB = _SB // 2
_FA, _FB = 256, 128
_F0 = _FA + _FB
_FU = (256, 128, 256, 256, 256, 256)
_FM = sum(_FU)
_OUT = (256, 128, 128)
_KM, _KR = 512, 64
_VR = 96


def _spans(sizes):
    out, off = [], 0
    for n in sizes:
        out.append((off, n))
        off += n
    return out


def _mm(a, b):
    return jnp.dot(a, b, preferred_element_type=_F32)


def _mm_nt(a, b):
    return lax.dot_general(a, b, (((1,), (1,)), ((), ())), preferred_element_type=_F32)


def _act2(g, u):
    t = jnp.tanh(g * (_C0 + _C1 * (g * g)))
    return ((g * (1.0 + t)) * u).astype(_BF16)


def _start(copies):
    for c in copies:
        c.start()


def _wait(copies):
    for c in copies:
        c.wait()


def _kernel(xT_hbm, wg_hbm, wu_hbm, wdT_hbm, oT_hbm,
            xT_v, x_v, wg0, wu0, wd0, wg, wu, wd, acc, o_v, xs, zs, zv, sem):
    n_chunks, n_blocks = x_v.shape[0], wg.shape[0]

    def copy(src, off, dst, s):
        return pltpu.make_async_copy(src.at[:, pl.ds(off, dst.shape[1])], dst, sem.at[s])

    def w_block(j, s):
        return [copy(src, _F0 + j * _FM, dst.at[j], s)
                for src, dst in ((wg_hbm, wg), (wu_hbm, wu), (wdT_hbm, wd))]

    def out_piece(c, off, n):
        dst = c * _SB + off
        if not isinstance(c, int):
            dst = pl.multiple_of(dst, 128)
        return pltpu.make_async_copy(
            o_v.at[c, :, pl.ds(off, n)], oT_hbm.at[:, pl.ds(dst, n)], sem.at[2])

    def transpose_x(c, off, n):
        x_v[c, off:off + n, :] = xT_v[c, :, off:off + n].T

    def gate_up(x, w_g, w_u):
        return _act2(_mm(x, w_g), _mm(x, w_u))

    def skew_x(c):
        xt = xT_v[c, _KM:, 0:128].astype(_F32)
        k = lax.broadcasted_iota(jnp.int32, (_KR, 128), 0)
        lane = lax.broadcasted_iota(jnp.int32, (_KR, 128), 1)
        for i in range(8):
            rel = lane - ((k - i) & 7)
            for r in range(_VR // 8):
                picked = jnp.sum(jnp.where(rel == 8 * r, xt, 0.0), axis=1, keepdims=True)
                xs[c, r, i] = jnp.broadcast_to(picked, (_KR, 128))

    def vpu_tail(c, w, prev):
        never = zv[...] != 0
        ws = [jnp.broadcast_to(w[8 * b:8 * b + 8], (2, 8, 128)) for b in range(_KR // 8)]
        rows = []
        for r in range(0, _VR // 8, 2):
            a = None
            for i in range(7, -1, -1):
                slab = xs[c, r:r + 2, i]
                if i % 2:
                    terms = [(b,) for b in range(8)]
                else:
                    terms = [(0, 1)] + [(b,) for b in range(2, 8)]
                for bs in terms:
                    p = None
                    for b in bs:
                        q = slab[:, 8 * b:8 * b + 8] * ws[b]
                        p = q if p is None else p + q
                    if a is not None:
                        a = a + p
                    elif prev[0] is not None:
                        a = jnp.where(never, prev[0], p)
                    else:
                        a = p
                if i:
                    a = pltpu.roll(a, 7, 1)
            prev[0] = a
            rows.append(a.reshape(16, 128))
        return jnp.concatenate(rows, axis=0)

    xa = copy(xT_hbm, 0, xT_v.at[0, :, pl.ds(0, _HB)], 0)
    ga = copy(wg_hbm, 0, wg0.at[:, pl.ds(0, _FA)], 1)
    ua = copy(wu_hbm, 0, wu0.at[:, pl.ds(0, _FA)], 2)
    in2 = [copy(xT_hbm, _HB, xT_v.at[0, :, pl.ds(_HB, _HB)], 0),
           copy(wg_hbm, _FA, wg0.at[:, pl.ds(_FA, _FB)], 0),
           copy(wu_hbm, _FA, wu0.at[:, pl.ds(_FA, _FB)], 0)]
    in3 = [copy(wdT_hbm, 0, wd0, 1), copy(xT_hbm, _SB, xT_v.at[1], 1)]
    in4 = [copy(xT_hbm, c * _SB, xT_v.at[c], 2) for c in range(2, n_chunks)]
    in5 = w_block(0, 0)
    in6 = [c for j in range(1, n_blocks) for c in w_block(j, 1)]

    _start([xa, ga, ua])
    zv[...] = jnp.zeros_like(zv)
    for i in range(zs.shape[0]):
        zs[i] = 0
    xa.wait()
    _start(in2)
    transpose_x(0, 0, _HB)
    ga.wait()
    _start(in3)
    g = jnp.concatenate([_mm(x_v[0, o:o + 128], wg0[:, :_FA]) for o in range(0, _HB, 128)], axis=0)
    ua.wait()
    u = jnp.concatenate([_mm(x_v[0, o:o + 128], wu0[:, :_FA]) for o in range(0, _HB, 128)], axis=0)
    h00 = _act2(g, u)
    _wait(in2)
    _start(in4)
    transpose_x(0, _HB, _HB)
    h01 = gate_up(x_v[0, :_HB], wg0[:, _FA:], wu0[:, _FA:])
    h1 = gate_up(x_v[0, _HB:], wg0[...], wu0[...])
    h = jnp.concatenate([jnp.concatenate([h00, h01], axis=1), h1], axis=0)
    _wait(in3)
    _start(in5)
    transpose_x(1, 0, _SB)
    acc[0] = _mm_nt(wd0[...], h)
    ha = gate_up(x_v[1], wg0[:, :_FA], wu0[:, :_FA])
    _wait(in4)
    _start(in6)
    for c in range(n_chunks):
        skew_x(c)
    for c in range(1, n_chunks):
        if c == 1:
            hb = [gate_up(x_v[c, o:o + _HB], wg0[:, _FA:], wu0[:, _FA:]) for o in (0, _HB)]
            h = jnp.concatenate([ha, jnp.concatenate(hb, axis=0)], axis=1)
        else:
            h = gate_up(x_v[c], wg0[...], wu0[...])
        if c + 1 < n_chunks:
            transpose_x(c + 1, 0, _SB)
        acc[c] = _mm_nt(wd0[...], h)
    _wait(in5)

    def body(it, carry):
        j, half = it >> 1, it & 1

        @pl.when(it == 1)
        def _():
            _wait(in6)

        prev, n_tiles = [None], [0]

        def project(c, w, off, n):
            main = _mm(x_v[c, :, :_KM], w[j, :_KM, off:off + n])
            tail = _mm(x_v[c, _VR:, _KM:], w[j, _KM:, off:off + n])
            tiles = []
            for t in range(off, off + n, 128):
                n_tiles[0] += 1
                tiles.append(w[j + zs[n_tiles[0] % zs.shape[0]], _KM:, t:t + 128].astype(_F32))
            return main, tail, tiles

        def hidden(c, off, n):
            gm, gt, gw = project(c, wg, off, n)
            um, ut, uw = project(c, wu, off, n)
            gv, uv = [], []
            for a, b in zip(gw, uw):
                gv.append(vpu_tail(c, a, prev))
                uv.append(vpu_tail(c, b, prev))
            g = gm + jnp.concatenate([jnp.concatenate(gv, axis=1), gt], axis=0)
            u = um + jnp.concatenate([jnp.concatenate(uv, axis=1), ut], axis=0)
            return _act2(g, u)

        def down(c, end, h, pieces):
            cols = slice(end - h.shape[1], end)
            if end < _FM:
                acc[c] += _mm_nt(wd[j, :, cols], h)
                return
            for so, sn in _spans(pieces):
                val = acc[c, :, so:so + sn] + _mm_nt(wd[j, :, cols], h[so:so + sn])
                acc[c, :, so:so + sn] = val
                o_v[c, :, so:so + sn] = (0.5 * val).astype(o_v.dtype)

                @pl.when(j == n_blocks - 1)
                def _():
                    out_piece(c, so, sn).start()

        pending = None
        for q, pieces in enumerate(((_SB,), _OUT)):
            c = 2 * half + q
            for off, n in _spans(_FU):
                h = hidden(c, off, n)
                if q == 1 and off + n == _FM:
                    h = jnp.concatenate([pending[2], h], axis=1)
                elif pending is not None:
                    down(*pending)
                pending = (c, off + n, h, pieces)
        down(*pending)
        return carry

    lax.fori_loop(0, 2 * n_blocks, body, 0)
    for c in range(n_chunks):
        _wait([out_piece(c, so, sn) for so, sn in _spans(_OUT if c % 2 else (_SB,))])


@jax.jit
def pallas_standalone__geglu_ffn__prompt_kernel(
    x: jax.Array,
    w_gate: jax.Array,
    w_up: jax.Array,
    w_down: jax.Array,
):
    B, S, D = x.shape
    F = w_gate.shape[1]
    T = B * S
    n_chunks, n_blocks = T // _SB, (F - _F0) // _FM
    assert T == 4 * _SB and F == _F0 + n_blocks * _FM and D == _KM + _KR
    scratch = (
        [pltpu.VMEM((n_chunks, D, _SB), _BF16), pltpu.VMEM((n_chunks, _SB, D), _BF16)]
        + [pltpu.VMEM((D, _F0), _BF16)] * 3
        + [pltpu.VMEM((n_blocks, D, _FM), _BF16)] * 3
        + [
            pltpu.VMEM((n_chunks, D, _SB), _F32),
            pltpu.VMEM((n_chunks, D, _SB), x.dtype),
            pltpu.VMEM((n_chunks, _VR // 8, 8, _KR, 128), _F32),
            pltpu.SMEM((16,), jnp.int32),
            pltpu.VMEM((2, 8, 128), jnp.int32),
            pltpu.SemaphoreType.DMA((3,)),
        ]
    )
    out_t = pl.pallas_call(
        _kernel,
        in_specs=[pl.BlockSpec(memory_space=pl.ANY)] * 4,
        out_specs=pl.BlockSpec(memory_space=pl.ANY),
        out_shape=jax.ShapeDtypeStruct((D, T), x.dtype),
        scratch_shapes=scratch,
        compiler_params=pltpu.CompilerParams(vmem_limit_bytes=64 * 1024 * 1024),
    )(x.reshape(T, D).T, w_gate, w_up, w_down.T)
    return out_t.T.reshape(B, S, D)
```
